```python
import jax
import jax.numpy as jnp

def _softmax(x, axis=-1):
    return jax.nn.softmax(x, axis=axis)

def _gelu(x):
    return jax.nn.gelu(x, approximate=True)

def _silu(x):
    return jax.nn.silu(x)

def _sigmoid(x):
    return jax.nn.sigmoid(x)

def _layernorm(x, axis=-1, eps=1e-05):
    m = jnp.mean(x, axis=axis, keepdims=True)
    v = jnp.var(x, axis=axis, keepdims=True)
    return (x - m) / jnp.sqrt(v + eps)

def _scatter_add(tgt, idx, src, axis=0):
    return tgt.at[idx].add(src)

def _segment_sum(src, seg, n):
    return jax.ops.segment_sum(src, seg, n)

class _Rng:

    def __init__(self, key):
        self._k = key

    def _next(self):
        self._k, sub = jax.random.split(self._k)
        return sub

    def normal(self, shape):
        return jax.random.normal(self._next(), shape, dtype=jnp.bfloat16)

    def randint(self, lo, hi, shape):
        return jax.random.randint(self._next(), shape, lo, hi, dtype=jnp.int32)

    def uniform(self, shape, lo=0.0, hi=1.0):
        return jax.random.uniform(self._next(), shape, jnp.bfloat16, lo, hi)

    def permutation(self, n):
        return jax.random.permutation(self._next(), n)
kernel_name = 'adaLN_cond__sliding_local_dilated__mixer_s_mlp__prompt'

def setup_inputs():
    _rng = _Rng(jax.random.key(int.from_bytes(__import__("os").urandom(4), "little")))
    _w = lambda a: (lambda t: t.astype(jnp.bfloat16) if jnp.issubdtype(t.dtype, jnp.floating) else t)(jnp.asarray(a))

    def _A_setup():
        B, S, D = (1, 2048, 1024)
        return {'x': _w((lambda *s: _rng.normal(s) * 0.05)(B, S, D)), 'wqkv': _w((lambda *s: _rng.normal(s) * 0.05)(D, 3 * D)), 'wo': _w((lambda *s: _rng.normal(s) * 0.05)(D, D))}
    _A_in = _A_setup()

    def _B_setup():
        B, S, D, F = (1, 2048, 1024, 3584)
        return {'x': _w((lambda *s: _rng.normal(s) * 0.05)(B, S, D)), 'w1': _w((lambda *s: _rng.normal(s) * 0.05)(D, D) * D ** (-0.5)), 'w2': _w((lambda *s: _rng.normal(s) * 0.05)(D, D) * D ** (-0.5)), 'w3': _w((lambda *s: _rng.normal(s) * 0.05)(D, F) * D ** (-0.5)), 'w4': _w((lambda *s: _rng.normal(s) * 0.05)(F, D) * F ** (-0.5))}
    _B_in = _B_setup()
    return {'A_x': _A_in['x'], 'A_wqkv': _A_in['wqkv'], 'A_wo': _A_in['wo'], 'B_x': _B_in['x'], 'B_w1': _B_in['w1'], 'B_w2': _B_in['w2'], 'B_w3': _B_in['w3'], 'B_w4': _B_in['w4'], 'c': _w((lambda *s: _rng.normal(s) * 0.05)(1, 1024)), 'w_mod': _w((lambda *s: _rng.normal(s) * 0.05)(1024, 6 * 1024) * 1024 ** (-0.5))}

def reference(A_x, A_wqkv, A_wo, B_x, B_w1, B_w2, B_w3, B_w4, c, w_mod):

    def _A_ref(x, wqkv, wo):
        B, S, D = x.shape
        H = 32
        Dh = D // H
        W, dil = (8, 2)
        qkv = (lambda x, *d: x.transpose(*d))((x @ wqkv).reshape(B, S, 3, H, Dh), 2, 0, 3, 1, 4)
        q, k, v = (qkv[0], qkv[1], qkv[2])
        scale = Dh ** (-0.5)
        pos = jnp.arange(S)
        off = jnp.arange(W) * dil
        idx = pos[:, None] - off[None, :]
        mask = idx >= 0
        idx_c = jnp.where(mask, idx, 0).reshape(-1)
        kg = k[:, :, idx_c, :].reshape(B, H, S, W, Dh)
        vg = v[:, :, idx_c, :].reshape(B, H, S, W, Dh)
        logits = jnp.einsum('bhsd,bhswd->bhsw', q, kg) * scale
        logits = jnp.where(mask[None, None, :, :], logits, -1000000000.0)
        attn = _softmax(logits, axis=-1)
        o = jnp.einsum('bhsw,bhswd->bhsd', attn, vg)
        return (lambda x, *d: x.transpose(*d))(o, 0, 2, 1, 3).reshape(B, S, D) @ wo

    def _B_ref(x, w1, w2, w3, w4):
        B, S, D = x.shape
        h = _gelu(_layernorm(x, axis=-1) @ w1)
        c = D // 4
        g0 = jnp.pad(h[:, :, 0 * c:1 * c], ((0, 0), (1, 0), (0, 0)))[:, :S, :]
        g1 = jnp.pad(h[:, :, 1 * c:2 * c], ((0, 0), (0, 1), (0, 0)))[:, 1:, :]
        g2 = jnp.pad(h[:, :, 2 * c:3 * c], ((0, 0), (2, 0), (0, 0)))[:, :S, :]
        g3 = jnp.pad(h[:, :, 3 * c:], ((0, 0), (0, 2), (0, 0)))[:, 2:, :]
        hs = jnp.concatenate([g0, g1, g2, g3], axis=-1) @ w2
        x1 = x + hs
        h2 = _gelu(_layernorm(x1, axis=-1) @ w3) @ w4
        return x1 + h2
    x = A_x
    mod = (_silu(c) @ w_mod).reshape(c.shape[0], 6, 1, -1)
    sa, ca, ga, sb, cb, gb = (mod[:, 0].copy(), mod[:, 1].copy(), mod[:, 2].copy(), mod[:, 3].copy(), mod[:, 4].copy(), mod[:, 5].copy())
    h = _layernorm(x, axis=-1) * (1 + ca) + sa
    x = x + ga * _A_ref(h, A_wqkv, A_wo)
    h = _layernorm(x, axis=-1) * (1 + cb) + sb
    x = x + gb * _B_ref(h, B_w1, B_w2, B_w3, B_w4)
    return x
```

```python
import jax
import jax.numpy as jnp
import jax.experimental.pallas as pl
import jax.experimental.pallas.tpu as pltpu

T = 256
FC = 512
DH = 32
W = 8
F32 = jnp.float32
BF = jnp.bfloat16


def _ln(x):
    m = jnp.mean(x, axis=-1, keepdims=True)
    d = x - m
    v = jnp.mean(d * d, axis=-1, keepdims=True)
    return d * jax.lax.rsqrt(v + 1e-5)


def _dot(a, b):
    return jnp.dot(a, b, preferred_element_type=F32)


def _kernel(x_ref, c_ref, wm_h, wqkv_h, wo_h, w1_h, w2_h, w3_h, w4_h, o_ref,
            wm, wqkv, wo, w1, w2, w3, w4, sems,
            mod, q_s, k_s, v_s, a_s, xp_s, g_s):
    i = pl.program_id(0)
    n = pl.num_programs(0) - 1
    D = x_ref.shape[1]
    F = w3.shape[1]
    cps = [pltpu.make_async_copy(s, d, sems.at[j]) for j, (s, d) in enumerate(
        [(wm_h, wm), (wqkv_h, wqkv), (wo_h, wo), (w1_h, w1), (w2_h, w2),
         (w3_h, w3), (w4_h, w4)])]

    @pl.when(i == 0)
    def _():
        for cp in cps[:2]:
            cp.start()
        k_s[0:16, :] = jnp.zeros((16, D), F32)
        v_s[0:16, :] = jnp.zeros((16, D), F32)
        g_s[0, 0:8, :] = jnp.zeros((8, D), F32)
        cps[0].wait()
        c = jnp.broadcast_to(c_ref[...].astype(F32), (8, D))
        mod[...] = _dot((c * jax.nn.sigmoid(c)).astype(BF), wm[...])
        cps[1].wait()
        for cp in cps[2:]:
            cp.start()

    def md(j):
        return mod[0:1, j * D:(j + 1) * D]

    slot = i % 2

    @pl.when(i < n)
    def _():
        x = x_ref[...].astype(F32)
        h = (_ln(x) * (1 + md(1)) + md(0)).astype(BF)
        q_s[...] = _dot(h, wqkv[:, 0:D]) * (DH ** -0.5)
        k_s[16:, :] = _dot(h, wqkv[:, D:2 * D])
        v_s[16:, :] = _dot(h, wqkv[:, 2 * D:])
        ri = jax.lax.broadcasted_iota(jnp.int32, (128, 128), 0) // DH
        ci = jax.lax.broadcasted_iota(jnp.int32, (128, 128), 1) // DH
        e = jnp.where(ri == ci, 1.0, 0.0).astype(BF)
        R = 128
        for r in range(T // R):
            row = jax.lax.broadcasted_iota(jnp.int32, (R, 128), 0) + (i * T + r * R)
            for g in range(D // 128):
                cs = slice(g * 128, (g + 1) * 128)
                q = q_s[r * R:(r + 1) * R, cs]
                ls = []
                for w in range(W):
                    b = 16 + r * R - 2 * w
                    l = _dot((q * k_s[b:b + R, cs]).astype(BF), e)
                    if w and r == 0:
                        l = jnp.where(row >= 2 * w, l, -1e9)
                    ls.append(l)
                m = ls[0]
                for l in ls[1:]:
                    m = jnp.maximum(m, l)
                den = acc = None
                for w in range(W):
                    b = 16 + r * R - 2 * w
                    p = jnp.exp(ls[w] - m)
                    pv = p * v_s[b:b + R, cs]
                    den = p if w == 0 else den + p
                    acc = pv if w == 0 else acc + pv
                a_s[r * R:(r + 1) * R, cs] = (acc / den).astype(BF)
        k_s[0:16, :] = k_s[T:T + 16, :]
        v_s[0:16, :] = v_s[T:T + 16, :]

        @pl.when(i == 0)
        def _():
            cps[2].wait()
            cps[3].wait()

        xp = x + md(2) * _dot(a_s[...], wo[...])
        xp_s[slot] = xp
        hb = _ln(xp) * (1 + md(4)) + md(3)
        g = jax.nn.gelu(_dot(_ln(hb).astype(BF), w1[...]), approximate=True)
        g_s[slot, 8:8 + T, :] = g
        g_s[1 - slot, 8 + T:, :] = g[0:8]

    @pl.when(i == n)
    def _():
        g_s[1 - slot, 8 + T:, :] = jnp.zeros((8, D), F32)

    @pl.when(i == 1)
    def _():
        for cp in cps[4:]:
            cp.wait()

    @pl.when(i > 0)
    def _():
        ps = 1 - slot
        c4 = D // 4
        hs = jnp.concatenate(
            [g_s[ps, 8 + o:8 + o + T, j * c4:(j + 1) * c4].astype(BF)
             for j, o in enumerate((-1, 1, -2, 2))], axis=-1)
        xp = xp_s[ps]
        hb = _ln(xp) * (1 + md(4)) + md(3)
        x1 = hb + _dot(hs, w2[...])
        hn = _ln(x1).astype(BF)
        acc = x1
        for f in range(F // FC):
            fs = slice(f * FC, (f + 1) * FC)
            u = jax.nn.gelu(_dot(hn, w3[:, fs]), approximate=True).astype(BF)
            acc = acc + _dot(u, w4[fs, :])
        o_ref[...] = (xp + md(5) * acc).astype(o_ref.dtype)

    @pl.when(i < n)
    def _():
        g_s[1 - slot, 0:8, :] = g_s[slot, T:T + 8, :]


@jax.jit
def pallas_adaLN_cond__sliding_local_dilated__mixer_s_mlp__prompt_kernel(
        A_x, A_wqkv, A_wo, B_x, B_w1, B_w2, B_w3, B_w4, c, w_mod):
    B, S, D = A_x.shape
    n = S // T
    ws = (w_mod, A_wqkv, A_wo, B_w1, B_w2, B_w3, B_w4)
    out = pl.pallas_call(
        _kernel,
        grid=(n + 1,),
        in_specs=[pl.BlockSpec((T, D), lambda i: (jnp.minimum(i, n - 1), 0)),
                  pl.BlockSpec((1, D), lambda i: (0, 0))]
        + [pl.BlockSpec(memory_space=pl.ANY)] * 7,
        out_specs=pl.BlockSpec((T, D), lambda i: (jnp.maximum(i - 1, 0), 0)),
        out_shape=jax.ShapeDtypeStruct((S, D), A_x.dtype),
        scratch_shapes=[pltpu.VMEM(w.shape, w.dtype) for w in ws] + [
            pltpu.SemaphoreType.DMA((7,)),
            pltpu.VMEM((8, 6 * D), F32),
            pltpu.VMEM((T, D), F32),
            pltpu.VMEM((T + 16, D), F32),
            pltpu.VMEM((T + 16, D), F32),
            pltpu.VMEM((T, D), BF),
            pltpu.VMEM((2, T, D), F32),
            pltpu.VMEM((2, T + 16, D), F32),
        ],
        compiler_params=pltpu.CompilerParams(
            dimension_semantics=("arbitrary",),
            vmem_limit_bytes=110 * 1024 * 1024),
    )(A_x.reshape(S, D), c, *ws)
    return out.reshape(B, S, D)
```

```python
import jax
import jax.numpy as jnp
import jax.experimental.pallas as pl
import jax.experimental.pallas.tpu as pltpu

T = 256
FC = 512
DH = 32
W = 8
F32 = jnp.float32
BF = jnp.bfloat16


def _ln(x):
    m = jnp.mean(x, axis=-1, keepdims=True)
    d = x - m
    v = jnp.mean(d * d, axis=-1, keepdims=True)
    return d * jax.lax.rsqrt(v + 1e-5)


def _dot(a, b):
    return jnp.dot(a, b, preferred_element_type=F32)


def _kernel(x_ref, c_ref, wm_h, wqkv_h, wo_h, w1_h, w2_h, w3_h, w4_h, o_ref,
            wm, wqkv, wo, w1, w2, w3, w4, sems,
            mod, q_s, k_s, v_s, a_s, xp_s, g_s):
    i = pl.program_id(0)
    n = pl.num_programs(0) - 1
    D = x_ref.shape[1]
    F = w3.shape[1]

    def cols(src, dst, lo, hi, j):
        return pltpu.make_async_copy(src.at[:, lo * D:hi * D],
                                     dst.at[:, lo * D:hi * D], sems.at[j])

    m_a = cols(wm_h, wm, 0, 2, 0)
    c_q = cols(wqkv_h, wqkv, 0, 1, 1)
    c_kv = cols(wqkv_h, wqkv, 1, 3, 2)
    m_b = cols(wm_h, wm, 2, 5, 3)
    c_o = pltpu.make_async_copy(wo_h, wo, sems.at[4])
    c_1 = pltpu.make_async_copy(w1_h, w1, sems.at[5])
    c_2 = pltpu.make_async_copy(w2_h, w2, sems.at[6])
    m_c = cols(wm_h, wm, 5, 6, 7)
    c_3 = pltpu.make_async_copy(w3_h, w3, sems.at[8])
    c_4 = pltpu.make_async_copy(w4_h, w4, sems.at[9])

    def modulation(lo, hi):
        c = jnp.broadcast_to(c_ref[...].astype(F32), (8, D))
        mod[:, lo * D:hi * D] = _dot((c * jax.nn.sigmoid(c)).astype(BF),
                                     wm[:, lo * D:hi * D])

    @pl.when(i == 0)
    def _():
        m_a.start()
        c_q.start()
        k_s[0:16, :] = jnp.zeros((16, D), F32)
        v_s[0:16, :] = jnp.zeros((16, D), F32)
        g_s[0, 0:8, :] = jnp.zeros((8, D), F32)
        m_a.wait()
        c_kv.start()
        modulation(0, 2)
        c_q.wait()
        m_b.start()
        c_o.start()
        c_1.start()

    def md(j):
        return mod[0:1, j * D:(j + 1) * D]

    slot = i % 2

    @pl.when(i < n)
    def _():
        x = x_ref[...].astype(F32)
        h = (_ln(x) * (1 + md(1)) + md(0)).astype(BF)
        q_s[...] = _dot(h, wqkv[:, 0:D]) * (DH ** -0.5)

        @pl.when(i == 0)
        def _():
            c_kv.wait()

        k_s[16:, :] = _dot(h, wqkv[:, D:2 * D])
        v_s[16:, :] = _dot(h, wqkv[:, 2 * D:])
        ri = jax.lax.broadcasted_iota(jnp.int32, (128, 128), 0) // DH
        ci = jax.lax.broadcasted_iota(jnp.int32, (128, 128), 1) // DH
        e = jnp.where(ri == ci, 1.0, 0.0).astype(BF)
        R = 128
        for r in range(T // R):
            row = jax.lax.broadcasted_iota(jnp.int32, (R, 128), 0) + (i * T + r * R)
            for g in range(D // 128):
                cs = slice(g * 128, (g + 1) * 128)
                q = q_s[r * R:(r + 1) * R, cs]
                ls = []
                for w in range(W):
                    b = 16 + r * R - 2 * w
                    l = _dot((q * k_s[b:b + R, cs]).astype(BF), e)
                    if w and r == 0:
                        l = jnp.where(row >= 2 * w, l, -1e9)
                    ls.append(l)
                m = ls[0]
                for l in ls[1:]:
                    m = jnp.maximum(m, l)
                den = acc = None
                for w in range(W):
                    b = 16 + r * R - 2 * w
                    p = jnp.exp(ls[w] - m)
                    pv = p * v_s[b:b + R, cs]
                    den = p if w == 0 else den + p
                    acc = pv if w == 0 else acc + pv
                a_s[r * R:(r + 1) * R, cs] = (acc / den).astype(BF)
        k_s[0:16, :] = k_s[T:T + 16, :]
        v_s[0:16, :] = v_s[T:T + 16, :]

        @pl.when(i == 0)
        def _():
            m_b.wait()
            c_o.wait()
            c_1.wait()
            for cp in (c_2, m_c, c_3, c_4):
                cp.start()
            modulation(2, 5)

        xp = x + md(2) * _dot(a_s[...], wo[...])
        xp_s[slot] = xp
        hb = _ln(xp) * (1 + md(4)) + md(3)
        g = jax.nn.gelu(_dot(_ln(hb).astype(BF), w1[...]), approximate=True)
        g_s[slot, 8:8 + T, :] = g
        g_s[1 - slot, 8 + T:, :] = g[0:8]

    @pl.when(i == n)
    def _():
        g_s[1 - slot, 8 + T:, :] = jnp.zeros((8, D), F32)

    @pl.when(i == 1)
    def _():
        for cp in (c_2, m_c, c_3, c_4):
            cp.wait()
        modulation(5, 6)

    @pl.when(i > 0)
    def _():
        ps = 1 - slot
        c4 = D // 4
        hs = jnp.concatenate(
            [g_s[ps, 8 + o:8 + o + T, j * c4:(j + 1) * c4].astype(BF)
             for j, o in enumerate((-1, 1, -2, 2))], axis=-1)
        xp = xp_s[ps]
        hb = _ln(xp) * (1 + md(4)) + md(3)
        x1 = hb + _dot(hs, w2[...])
        hn = _ln(x1).astype(BF)
        acc = x1
        for f in range(F // FC):
            fs = slice(f * FC, (f + 1) * FC)
            u = jax.nn.gelu(_dot(hn, w3[:, fs]), approximate=True).astype(BF)
            acc = acc + _dot(u, w4[fs, :])
        o_ref[...] = (xp + md(5) * acc).astype(o_ref.dtype)

    @pl.when(i < n)
    def _():
        g_s[1 - slot, 0:8, :] = g_s[slot, T:T + 8, :]


@jax.jit
def pallas_adaLN_cond__sliding_local_dilated__mixer_s_mlp__prompt_kernel(
        A_x, A_wqkv, A_wo, B_x, B_w1, B_w2, B_w3, B_w4, c, w_mod):
    B, S, D = A_x.shape
    n = S // T
    ws = (w_mod, A_wqkv, A_wo, B_w1, B_w2, B_w3, B_w4)
    out = pl.pallas_call(
        _kernel,
        grid=(n + 1,),
        in_specs=[pl.BlockSpec((T, D), lambda i: (jnp.minimum(i, n - 1), 0)),
                  pl.BlockSpec((1, D), lambda i: (0, 0))]
        + [pl.BlockSpec(memory_space=pl.ANY)] * 7,
        out_specs=pl.BlockSpec((T, D), lambda i: (jnp.maximum(i - 1, 0), 0)),
        out_shape=jax.ShapeDtypeStruct((S, D), A_x.dtype),
        scratch_shapes=[pltpu.VMEM(w.shape, w.dtype) for w in ws] + [
            pltpu.SemaphoreType.DMA((10,)),
            pltpu.VMEM((8, 6 * D), F32),
            pltpu.VMEM((T, D), F32),
            pltpu.VMEM((T + 16, D), F32),
            pltpu.VMEM((T + 16, D), F32),
            pltpu.VMEM((T, D), BF),
            pltpu.VMEM((2, T, D), F32),
            pltpu.VMEM((2, T + 16, D), F32),
        ],
        compiler_params=pltpu.CompilerParams(
            dimension_semantics=("arbitrary",),
            vmem_limit_bytes=110 * 1024 * 1024),
    )(A_x.reshape(S, D), c, *ws)
    return out.reshape(B, S, D)
```
